```python
import jax
import jax.numpy as jnp

def _softmax(x, axis=-1):
    return jax.nn.softmax(x, axis=axis)

def _gelu(x):
    return jax.nn.gelu(x, approximate=True)

def _silu(x):
    return jax.nn.silu(x)

def _sigmoid(x):
    return jax.nn.sigmoid(x)

def _layernorm(x, axis=-1, eps=1e-05):
    m = jnp.mean(x, axis=axis, keepdims=True)
    v = jnp.var(x, axis=axis, keepdims=True)
    return (x - m) / jnp.sqrt(v + eps)

def _scatter_add(tgt, idx, src, axis=0):
    return tgt.at[idx].add(src)

def _segment_sum(src, seg, n):
    return jax.ops.segment_sum(src, seg, n)

class _Rng:

    def __init__(self, key):
        self._k = key

    def _next(self):
        self._k, sub = jax.random.split(self._k)
        return sub

    def normal(self, shape):
        return jax.random.normal(self._next(), shape, dtype=jnp.bfloat16)

    def randint(self, lo, hi, shape):
        return jax.random.randint(self._next(), shape, lo, hi, dtype=jnp.int32)

    def uniform(self, shape, lo=0.0, hi=1.0):
        return jax.random.uniform(self._next(), shape, jnp.bfloat16, lo, hi)

    def permutation(self, n):
        return jax.random.permutation(self._next(), n)
kernel_name = 'interleave_layers__linear_kernel_hedgehog__mixer_gmlp__prompt'

def _fwd_setup_inputs():
    _rng = _Rng(jax.random.key(int.from_bytes(__import__("os").urandom(4), "little")))
    _w = lambda a: (lambda t: t.astype(jnp.bfloat16) if jnp.issubdtype(t.dtype, jnp.floating) else t)(jnp.asarray(a))

    def _A_setup():
        B, S, D, H = (1, 2048, 640, 32)
        Dh = D // H
        return {'x': _w((lambda *s: _rng.normal(s) * 0.05)(B, S, D)), 'wqkv': _w((lambda *s: _rng.normal(s) * 0.05)(D, 3 * D)), 'w_phi': _w((lambda *s: _rng.normal(s) * 0.05)(H, Dh, Dh) * Dh ** (-0.5)), 'wo': _w((lambda *s: _rng.normal(s) * 0.05)(D, D))}
    _A_in = _A_setup()

    def _B_setup():
        B, S, D, F = (1, 2048, 640, 1536)
        Fh = F // 2
        return {'x': _w((lambda *s: _rng.normal(s) * 0.05)(B, S, D)), 'w_in': _w((lambda *s: _rng.normal(s) * 0.05)(D, 2 * Fh)), 'w_sp': _w(0.01 * (lambda *s: _rng.normal(s) * 0.05)(S, S)), 'b_sp': _w(1.0 + 0.01 * (lambda *s: _rng.normal(s) * 0.05)(S)), 'w_out': _w((lambda *s: _rng.normal(s) * 0.05)(Fh, D))}
    _B_in = _B_setup()
    return {'A_x': _A_in['x'], 'A_wqkv': _A_in['wqkv'], 'A_w_phi': _A_in['w_phi'], 'A_wo': _A_in['wo'], 'B_x': _B_in['x'], 'B_w_in': _B_in['w_in'], 'B_w_sp': _B_in['w_sp'], 'B_b_sp': _B_in['b_sp'], 'B_w_out': _B_in['w_out']}

def _fwd_reference(A_x, A_wqkv, A_w_phi, A_wo, B_x, B_w_in, B_w_sp, B_b_sp, B_w_out):

    def _A_ref(x, wqkv, w_phi, wo):
        B, S, D = x.shape
        H = 32
        Dh = D // H
        qkv = (lambda x, *d: x.transpose(*d))((x @ wqkv).reshape(B, S, 3, H, Dh), 2, 0, 3, 1, 4)
        q, k, v = (qkv[0], qkv[1], qkv[2])
        pq = jnp.einsum('bhsd,hdf->bhsf', q, w_phi)
        pk = jnp.einsum('bhsd,hdf->bhsf', k, w_phi)
        phi_q = jnp.concatenate([_softmax(pq, axis=-1), _softmax(-pq, axis=-1)], axis=-1)
        phi_k = jnp.concatenate([_softmax(pk, axis=-1), _softmax(-pk, axis=-1)], axis=-1)
        kv = jnp.einsum('bhsf,bhsd->bhfd', phi_k, v)
        z = jnp.einsum('bhsf->bhf', phi_k)
        num = jnp.einsum('bhqf,bhfd->bhqd', phi_q, kv)
        den = jnp.einsum('bhqf,bhf->bhq', phi_q, z)[..., None] + 1e-06
        o = num / den
        return (lambda x, *d: x.transpose(*d))(o, 0, 2, 1, 3).reshape(B, S, D) @ wo

    def _B_ref(x, w_in, w_sp, b_sp, w_out):
        B, S, D = x.shape
        F = w_in.shape[-1]
        Fh = F // 2
        z = _gelu(jnp.einsum('bsd,df->bsf', x, w_in))
        z1 = z[..., :Fh].copy()
        z2 = _layernorm(z[..., Fh:], axis=-1)
        g = jnp.einsum('ts,bsf->btf', w_sp, z2) + b_sp[None, :, None]
        return jnp.einsum('bsf,fd->bsd', z1 * g, w_out)
    x = A_x
    x = x + _A_ref(_layernorm(x, axis=-1), A_wqkv, A_w_phi, A_wo)
    x = x + _B_ref(_layernorm(x, axis=-1), B_w_in, B_w_sp, B_b_sp, B_w_out)
    x = x + _A_ref(_layernorm(x, axis=-1), A_wqkv, A_w_phi, A_wo)
    x = x + _B_ref(_layernorm(x, axis=-1), B_w_in, B_w_sp, B_b_sp, B_w_out)
    return x

def setup_inputs():
    _inp = _fwd_setup_inputs()
    _gk = jax.random.fold_in(jax.random.key(int.from_bytes(__import__("os").urandom(4), "little")), 2 ** 31 - 1)
    _shapes = [[1, 2048, 640]]
    _dtypes = ['bfloat16']
    _gks = jax.random.split(_gk, len(_shapes))
    _gs = [jax.random.normal(k, s, dtype=jnp.dtype(d)) * 0.05 for k, s, d in zip(_gks, _shapes, _dtypes)]
    _inp['grad_out'] = _gs[0]
    return _inp

def reference(A_x, A_wqkv, A_w_phi, A_wo, B_w_in, B_w_sp, B_b_sp, B_w_out, B_x, grad_out):
    _const = dict(B_x=B_x)

    def _f(*_d):
        return _fwd_reference(**{'A_x': _d[0], 'A_wqkv': _d[1], 'A_w_phi': _d[2], 'A_wo': _d[3], 'B_w_in': _d[4], 'B_w_sp': _d[5], 'B_b_sp': _d[6], 'B_w_out': _d[7], **_const})
    _out, _vjp = jax.vjp(_f, A_x, A_wqkv, A_w_phi, A_wo, B_w_in, B_w_sp, B_b_sp, B_w_out)
    _grads = _vjp(grad_out)
    _out0 = jnp.asarray(_out)
    return (_out0, *[jnp.asarray(_g) for _g in _grads])
```

```python
import jax
import jax.numpy as jnp
import jax.experimental.pallas as pl
import jax.experimental.pallas.tpu as pltpu
from jax import lax

S, D, H, DH, F, FH = 2048, 640, 32, 20, 1536, 768
T = 512
NB = S // T
G = 4
GR = 160
GE = 176
GP = 320
f32, bf16 = jnp.float32, jnp.bfloat16


def _nn(a, b):
    return lax.dot_general(a, b, (((1,), (0,)), ((), ())), preferred_element_type=f32)


def _nt(a, b):
    return lax.dot_general(a, b, (((1,), (1,)), ((), ())), preferred_element_type=f32)


def _iota(shape, d):
    return lax.broadcasted_iota(jnp.int32, shape, d)


def _ln(x):
    m = jnp.mean(x, axis=0, keepdims=True)
    xc = x - m
    r = lax.rsqrt(jnp.mean(xc * xc, axis=0, keepdims=True) + 1e-5)
    return xc * r, r


def _ln_bwd(dn, n, r):
    return r * (dn - jnp.mean(dn, axis=0, keepdims=True)
                - n * jnp.mean(dn * n, axis=0, keepdims=True))


def _phi(p):
    p = p.reshape(DH, 8, T)
    ep = jnp.exp(p - jnp.max(p, axis=0, keepdims=True))
    em = jnp.exp(jnp.min(p, axis=0, keepdims=True) - p)
    ep = ep * (1.0 / jnp.sum(ep, axis=0, keepdims=True))
    em = em * (1.0 / jnp.sum(em, axis=0, keepdims=True))
    return jnp.concatenate([ep.reshape(GR, T), em.reshape(GR, T)], axis=0)


def _phi_bwd(dphi, phi):
    dphi = dphi.reshape(2, DH, 8, T)
    phi = phi.astype(f32).reshape(2, DH, 8, T)
    d = phi * (dphi - jnp.sum(phi * dphi, axis=1, keepdims=True))
    return (d[0] - d[1]).reshape(GR, T)


_C0 = 0.7978845608028654
_C1 = 0.044715


def _kernel(x_h, wqkv_h, wphi_ref, wo_h, win_h, wsp_h, bsp_ref, wout_h, go_h,
            out_h, dx_h, dwqkv_h, dwphi_ref, dwo_h, dwin_h, dwsp_h, db_ref, dwout_h, spill_h,
            xin, xs, wraw, bd, bdT, wT, wN, woraw, woT, woN, winN, winT, woutN, woutT, wsp,
            act, z1s, gs, z2s, dgs, dgT, dpq, rden, rstd, kvacc, kvT, kvN, dkvT, dkvN,
            dW, dWo, dWin, dWout, dbacc, ostg, pstg, lsem, osem, psem, ssem, wsem):
    N0, K0, V0 = 0, 640, 1920
    Q0, O0, M0, P0 = 2560, 3840, 4480, 5120
    END = 6656

    loads = [pltpu.make_async_copy(s, d, lsem.at[i]) for i, (s, d) in enumerate([
        (wqkv_h, wraw), (x_h, xin), (wo_h, woraw), (win_h, winN), (wout_h, woutN), (wsp_h, wsp)])]
    loads[0].start()
    loads[1].start()

    r_i, c_i = _iota((D, 128), 0), _iota((8, D), 1)
    r_h = jnp.tile(r_i // DH, (1, D // 128))
    r_f = jnp.tile(r_i % DH, (1, D // 128))
    c_h = jnp.tile((c_i // GR) * 8 + c_i % 8, (D // 8, 1))
    c_f = jnp.tile((c_i % GR) // 8, (D // 8, 1))
    same_head = r_h == c_h
    e_f = (_iota((128, D), 0) == c_f[:128]).astype(bf16)
    wphi = jnp.where(_iota((D, 128), 1) < DH, wphi_ref[...], jnp.zeros((), bf16))
    bd[0] = jnp.where(same_head, _nn(wphi, e_f), 0.0).astype(bf16)
    bd[1] = (same_head & (r_f == c_f)).astype(bf16)
    KLO = (0, 128, 256, 384)

    loads[0].wait()
    for c in loads[2:]:
        c.start()
    for j in range(2):
        bdT[j] = bd[j].astype(f32).T.astype(bf16)
    for j in range(3):
        for g in range(G):
            wT[j * D + g * GR:j * D + (g + 1) * GR, :] = _nt(
                bdT[j // 2, g * GR:(g + 1) * GR, KLO[g]:KLO[g] + 256],
                wraw[:, j * D + KLO[g]:j * D + KLO[g] + 256]).astype(bf16)
    loads[1].wait()

    ones_blk = (_iota((16, T), 0) < 8).astype(bf16)
    zeros8 = jnp.zeros((8, T), f32)
    kv_mask = (_iota((GE, GP), 0) % 8) == (_iota((GE, GP), 1) % 8)

    def loop(fn):
        lax.fori_loop(0, NB, lambda i, c: (fn(i), c)[1], 0)

    def fin_kv(dst_t, dst_n):
        for g in range(G):
            m = jnp.where(kv_mask, kvacc[g], 0.0)
            dst_t[g] = m.astype(bf16)
            dst_n[g] = m.T.astype(bf16)

    def a1(l, i, x):
        n, r = _ln(x)
        nb = n.astype(bf16)
        act[i, N0:N0 + D] = nb
        rstd[l, 0, i] = r
        pqkv = _nn(wT[...], nb)
        v = pqkv[2 * D:].astype(bf16)
        act[i, V0:V0 + D] = v
        for g in range(G):
            act[i, Q0 + g * GP:Q0 + (g + 1) * GP] = _phi(pqkv[g * GR:(g + 1) * GR]).astype(bf16)
            pk = _phi(pqkv[D + g * GR:D + (g + 1) * GR]).astype(bf16)
            act[i, K0 + g * GP:K0 + (g + 1) * GP] = pk
            vext = jnp.concatenate([v[g * GR:(g + 1) * GR], ones_blk], axis=0)
            kvacc[g] += _nt(vext, pk)

    def a2b1(l, i):
        os_, rs = [], []
        for g in range(G):
            nd = _nn(kvT[l, g], act[i, Q0 + g * GP:Q0 + (g + 1) * GP])
            rd = 1.0 / (nd[GR:GR + 8] + 1e-6)
            rs.append(rd)
            os_.append((nd[:GR].reshape(DH, 8, T) * rd[None]).reshape(GR, T).astype(bf16))
        o = jnp.concatenate(os_, axis=0)
        rden[l, i] = jnp.concatenate(rs, axis=0)
        act[i, O0:O0 + D] = o
        x1 = xs[i] + _nn(woT[...], o)
        xs[i] = x1
        n, r = _ln(x1)
        nb = n.astype(bf16)
        act[i, M0:M0 + D] = nb
        rstd[l, 1, i] = r
        u = _nn(winT[...], nb)
        u2 = u * u
        t = jnp.tanh(u * (_C0 + (_C0 * _C1) * u2))
        h = 0.5 * t + 0.5
        z = u * h
        act[i, P0:P0 + F] = (h + (0.5 * u) * (1.0 - t * t) * (_C0 + (3 * _C0 * _C1) * u2)).astype(bf16)
        z1s[l, i] = z[:FH].astype(bf16)
        z2, r2 = _ln(z[FH:])
        z2s[l, i] = z2.astype(bf16)
        rstd[l, 2, i] = r2

    def b2(l, i):
        t0 = pl.multiple_of(i * T, T)
        g = bsp_ref[i].astype(f32)
        for k in range(NB):
            g = g + _nt(z2s[l, k], wsp[pl.ds(t0, T), k * T:(k + 1) * T])
        y = (z1s[l, i].astype(f32) * g).astype(bf16)
        return xs[i] + _nn(woutT[...], y), g, y

    def b2_bwd(l, i, dx, g, y):
        dxb = dx.astype(bf16)
        dWout[...] += _nt(y, dxb)
        dy = _nn(woutN[...], dxb)
        dg = dy * z1s[l, i].astype(f32)
        z1s[l, i] = (dy * g).astype(bf16)
        dgs[i] = dg.astype(bf16)
        dgt = dg.T.astype(bf16)
        dsum = jnp.sum(dg, axis=0, keepdims=True)
        if l == 1:
            dgT[i] = dgt
            dbacc[i] = dsum
        else:
            db_ref[i] = (dbacc[i] + dsum).astype(bf16)
            slot = i % 2
            dgT[NB] = dgt

            def col(k, c_):
                pstg[slot, :, pl.ds(pl.multiple_of(k * T, T), T)] = (
                    _nn(dgT[i], z2s[1, k]) + _nn(dgT[NB], z2s[0, k])).astype(bf16)
                return c_
            lax.fori_loop(0, NB, col, 0)
            pltpu.make_async_copy(pstg.at[slot], dwsp_h.at[pl.ds(pl.multiple_of(i * T, T), T)],
                                  psem.at[slot]).start()

    def q2(l, i):
        t0 = pl.multiple_of(i * T, T)
        dz2 = _nn(dgs[0], wsp[0:T, pl.ds(t0, T)])
        for k in range(1, NB):
            dz2 = dz2 + _nn(dgs[k], wsp[k * T:(k + 1) * T, pl.ds(t0, T)])
        dz2 = _ln_bwd(dz2, z2s[l, i].astype(f32), rstd[l, 2, i])
        dz = jnp.concatenate([z1s[l, i].astype(f32), dz2], axis=0)
        du = (dz * act[i, P0:P0 + F].astype(f32)).astype(bf16)
        nb = act[i, M0:M0 + D]
        dWin[...] += _nt(nb, du)
        dx = xs[i] + _ln_bwd(_nn(winN[...], du), nb.astype(f32), rstd[l, 1, i])
        xs[i] = dx

    def q2b(l, i):
        dxb = xs[i].astype(bf16)
        o = act[i, O0:O0 + D]
        dWo[...] += _nt(o, dxb)
        do = _nn(woN[...], dxb)
        rd = rden[l, i]
        for g in range(G):
            rg = rd[g * 8:(g + 1) * 8]
            dog = do[g * GR:(g + 1) * GR].reshape(DH, 8, T)
            og = o[g * GR:(g + 1) * GR].astype(f32).reshape(DH, 8, T)
            dden = -jnp.sum(dog * og, axis=0) * rg
            ext = jnp.concatenate([(dog * rg[None]).reshape(GR, T), dden, zeros8], axis=0).astype(bf16)
            pq = act[i, Q0 + g * GP:Q0 + (g + 1) * GP]
            kvacc[g] += _nt(ext, pq)
            dpq[i, g * GR:(g + 1) * GR] = _phi_bwd(_nn(kvN[l, g], ext), pq).astype(bf16)


    def q1(l, i):
        dpk, dv = [], []
        for g in range(G):
            pk = act[i, K0 + g * GP:K0 + (g + 1) * GP]
            vext = jnp.concatenate([act[i, V0 + g * GR:V0 + (g + 1) * GR], ones_blk], axis=0)
            dpk.append(_phi_bwd(_nn(dkvN[g], vext), pk).astype(bf16))
            dv.append(_nn(dkvT[g, :GR], pk).astype(bf16))
        d = jnp.concatenate([dpq[i]] + dpk + dv, axis=0)
        nb = act[i, N0:N0 + D]
        dW[...] += _nt(nb, d)
        return xs[i] + _ln_bwd(_nn(wN[...], d), nb.astype(f32), rstd[l, 0, i])

    def emit_rows(dst, i, val):
        slot = i % 2
        ostg[slot] = val.T.astype(bf16)
        pltpu.make_async_copy(ostg.at[slot], dst.at[pl.ds(pl.multiple_of(i * T, T), T)],
                              osem.at[slot]).start()

    def free_slot(stg, dst, sem, i):
        @pl.when(i >= 2)
        def _():
            pltpu.make_async_copy(stg.at[i % 2], dst.at[pl.ds(0, T)], sem.at[i % 2]).wait()

    def drain(stg, dst, sem):
        for s_ in range(2):
            pltpu.make_async_copy(stg.at[s_], dst.at[pl.ds(0, T)], sem.at[s_]).wait()

    def rows_in(i):
        return xin[pl.ds(pl.multiple_of(i * T, T), T), :].astype(f32).T

    def spill(a, b, k, back):
        v, h = act.at[:, a:b], spill_h.at[:, a:b]
        return pltpu.make_async_copy(h, v, ssem.at[k]) if back else pltpu.make_async_copy(v, h, ssem.at[k])

    kvacc[...] = jnp.zeros_like(kvacc)

    def p1(i):
        x = rows_in(i)
        xs[i] = x
        a1(0, i, x)
    loop(p1)
    go_load = pltpu.make_async_copy(go_h, xin, lsem.at[1])
    go_load.start()
    c = spill(0, O0, 0, False)
    c.start()
    fin_kv(kvT.at[0], kvN.at[0])
    loads[2].wait()
    w = _nn(bdT[1], woraw[...])
    woN[...] = w.astype(bf16)
    woT[...] = w.T.astype(bf16)
    loads[3].wait()
    winT[...] = winN[...].astype(f32).T.astype(bf16)
    loads[4].wait()
    woutT[...] = woutN[...].astype(f32).T.astype(bf16)
    kvacc[...] = jnp.zeros_like(kvacc)

    def p2z(i):
        a2b1(0, i)
        for ref in (dW, dWo, dWin, dWout):
            n = ref.shape[0] // NB
            ref[pl.ds(pl.multiple_of(i * n, 8), n), :] = jnp.zeros((n, ref.shape[1]), f32)
    loop(p2z)
    loads[5].wait()
    c.wait()
    c = spill(O0, END, 1, False)
    c.start()

    def p31(i):
        x, g, _ = b2(0, i)
        gs[i] = g.astype(bf16)
        xs[i] = x
        a1(1, i, x)
    loop(p31)
    fin_kv(kvT.at[1], kvN.at[1])
    c.wait()
    loop(lambda i: a2b1(1, i))
    wN[...] = wT[...].astype(f32).T.astype(bf16)
    go_load.wait()

    def p3q3(i):
        free_slot(ostg, out_h, osem, i)
        x, g, y = b2(1, i)
        emit_rows(out_h, i, x)
        dx = rows_in(i)
        xs[i] = dx
        b2_bwd(1, i, dx, g, y)
    loop(p3q3)
    drain(ostg, out_h, osem)
    kvacc[...] = jnp.zeros_like(kvacc)
    loop(lambda i: q2(1, i))
    loop(lambda i: q2b(1, i))
    c = spill(Q0, END, 0, True)
    c.start()
    fin_kv(dkvT, dkvN)

    def q1q3(i):
        free_slot(pstg, dwsp_h, psem, i)
        dx = q1(1, i)
        xs[i] = dx
        g = gs[i].astype(f32)
        b2_bwd(0, i, dx, g, (z1s[0, i].astype(f32) * g).astype(bf16))
    loop(q1q3)
    drain(pstg, dwsp_h, psem)
    c.wait()
    c = spill(0, Q0, 1, True)
    c.start()
    woutN[...] = dWout[...].astype(bf16)
    cw = [pltpu.make_async_copy(woutN, dwout_h, wsem.at[0])]
    cw[-1].start()
    kvacc[...] = jnp.zeros_like(kvacc)
    loop(lambda i: q2(0, i))
    loop(lambda i: q2b(0, i))
    fin_kv(dkvT, dkvN)
    winN[...] = dWin[...].astype(bf16)
    cw.append(pltpu.make_async_copy(winN, dwin_h, wsem.at[1]))
    cw[-1].start()
    woN[...] = _nn(bd[1], dWo[...].astype(bf16)).astype(bf16)
    cw.append(pltpu.make_async_copy(woN, dwo_h, wsem.at[2]))
    cw[-1].start()
    c.wait()

    def q1last(i):
        free_slot(ostg, dx_h, osem, i)
        emit_rows(dx_h, i, q1(0, i))
    loop(q1last)

    PR = ((0, 256), (0, 384), (128, 512), (256, 640), (384, 640))
    dwb = [dW[:, j * D:(j + 1) * D].astype(bf16) for j in range(3)]
    for j in range(3):
        for c_, (lo_, hi_) in enumerate(PR):
            wN[:, j * D + c_ * 128:j * D + (c_ + 1) * 128] = _nt(
                dwb[j][:, lo_:hi_], bd[j // 2, c_ * 128:(c_ + 1) * 128, lo_:hi_]).astype(bf16)
    cw.append(pltpu.make_async_copy(wN, dwqkv_h, wsem.at[3]))
    cw[-1].start()
    for c_, (lo_, hi_) in enumerate(PR):
        acc = sum(lax.dot_general(wraw[:, j * D + c_ * 128:j * D + (c_ + 1) * 128], dwb[j][:, lo_:hi_],
                                  (((0,), (0,)), ((), ())), preferred_element_type=f32) for j in range(2))
        acc = jnp.where(same_head[c_ * 128:(c_ + 1) * 128, lo_:hi_], acc, 0.0)
        hi = acc.astype(bf16)
        lo = (acc - hi.astype(f32)).astype(bf16)
        e = e_f[:, lo_:hi_]
        dwphi_ref[c_ * 128:(c_ + 1) * 128, :] = (_nt(hi, e) + _nt(lo, e)).astype(bf16)
    drain(ostg, dx_h, osem)
    for c in cw:
        c.wait()


@jax.jit
def pallas_interleave_layers__linear_kernel_hedgehog__mixer_gmlp__prompt_kernel(
    A_x: jax.Array,
    A_wqkv: jax.Array,
    A_w_phi: jax.Array,
    A_wo: jax.Array,
    B_x: jax.Array,
    B_w_in: jax.Array,
    B_w_sp: jax.Array,
    B_b_sp: jax.Array,
    B_w_out: jax.Array,
    grad_out: jax.Array,
):
    del B_x
    sds = jax.ShapeDtypeStruct
    hbm = pl.BlockSpec(memory_space=pl.ANY)
    vm = pl.BlockSpec(memory_space=pltpu.VMEM)
    V = pltpu.VMEM
    dma = pltpu.SemaphoreType.DMA
    scratch = [
        V((S, D), bf16), V((NB, D, T), f32), V((D, 3 * D), bf16), V((2, D, D), bf16), V((2, D, D), bf16),
        V((3 * D, D), bf16), V((D, 3 * D), bf16), V((D, D), bf16), V((D, D), bf16), V((D, D), bf16),
        V((D, F), bf16), V((F, D), bf16), V((FH, D), bf16), V((D, FH), bf16), V((S, S), bf16),
        V((NB, 6656, T), bf16), V((2, NB, FH, T), bf16), V((NB, FH, T), bf16), V((2, NB, FH, T), bf16),
        V((NB, FH, T), bf16), V((NB + 1, T, FH), bf16), V((NB, D, T), bf16),
        V((2, NB, H, T), f32), V((2, 3, NB, 1, T), f32),
        V((G, GE, GP), f32), V((2, G, GE, GP), bf16), V((2, G, GP, GE), bf16),
        V((G, GE, GP), bf16), V((G, GP, GE), bf16),
        V((D, 3 * D), f32), V((D, D), f32), V((D, F), f32), V((FH, D), f32), V((NB, 1, T), f32),
        V((2, T, D), bf16), V((2, T, S), bf16),
        dma((6,)), dma((2,)), dma((2,)), dma((2,)), dma((4,)),
    ]
    outs = pl.pallas_call(
        _kernel,
        in_specs=[hbm, hbm, vm, hbm, hbm, hbm, vm, hbm, hbm],
        out_specs=[hbm, hbm, hbm, vm, hbm, hbm, hbm, vm, hbm, hbm],
        out_shape=[sds((S, D), bf16), sds((S, D), bf16), sds((D, 3 * D), bf16), sds((D, 128), bf16),
                   sds((D, D), bf16), sds((D, F), bf16), sds((S, S), bf16), sds((NB, 1, T), bf16),
                   sds((FH, D), bf16), sds((NB, 6656, T), bf16)],
        scratch_shapes=scratch,
        compiler_params=pltpu.CompilerParams(vmem_limit_bytes=127 * 1024 * 1024),
    )(A_x.reshape(S, D), A_wqkv, jnp.pad(A_w_phi.reshape(D, DH), ((0, 0), (0, 128 - DH))), A_wo,
      B_w_in, B_w_sp, B_b_sp.reshape(NB, 1, T), B_w_out, grad_out.reshape(S, D))
    out, dx, dwqkv, dwphi, dwo, dwin, dwsp, db, dwout, _ = outs
    return (out.reshape(1, S, D), dx.reshape(1, S, D), dwqkv, dwphi[:, :DH].reshape(H, DH, DH),
            dwo, dwin, dwsp, db.reshape(S), dwout)
```
